```python
import jax
import jax.numpy as jnp

def _softmax(x, axis=-1):
    return jax.nn.softmax(x, axis=axis)
def _gelu(x):
    return jax.nn.gelu(x, approximate=True)
def _silu(x):
    return jax.nn.silu(x)
def _sigmoid(x):
    return jax.nn.sigmoid(x)
def _layernorm(x, axis=-1, eps=1e-5):
    m = jnp.mean(x, axis=axis, keepdims=True)
    v = jnp.var(x, axis=axis, keepdims=True)
    return (x - m) / jnp.sqrt(v + eps)
def _scatter_add(tgt, idx, src, axis=0):
    return tgt.at[idx].add(src)
def _segment_sum(src, seg, n):
    return jax.ops.segment_sum(src, seg, n)
class _Rng:
    def __init__(self, key):
        self._k = key
    def _next(self):
        self._k, sub = jax.random.split(self._k)
        return sub
    def normal(self, shape):
        return jax.random.normal(self._next(), shape, dtype=jnp.bfloat16)
    def randint(self, lo, hi, shape):
        return jax.random.randint(self._next(), shape, lo, hi, dtype=jnp.int32)
    def uniform(self, shape, lo=0.0, hi=1.0):
        return jax.random.uniform(self._next(), shape, jnp.bfloat16, lo, hi)
    def permutation(self, n):
        return jax.random.permutation(self._next(), n)


kernel_name = 'concat_heads__ssm_conv_h3__linear_attn_block__prompt'

def setup_inputs():
    _rng = _Rng(jax.random.key(int.from_bytes(__import__("os").urandom(4), "little")))
    _w = (lambda a: (lambda t: t.astype(jnp.bfloat16) if jnp.issubdtype(t.dtype, jnp.floating) else t)(jnp.asarray(a)))
    def _A_setup():
        B, S, D = 1, 2048, 1024
        ks = 4
        return {
            "q": _w((lambda *s: _rng.normal(s) * 0.05)(B, S, D)),
            "k": _w((lambda *s: _rng.normal(s) * 0.05)(B, S, D)),
            "v": _w((lambda *s: _rng.normal(s) * 0.05)(B, S, D)),
            "shift_k": _w((lambda *s: _rng.normal(s) * 0.05)(D, ks) * 0.5),
            "ssm_k": _w((lambda *s: _rng.normal(s) * 0.05)(D, S) * (1.0 / S ** 0.5)),
            "ssm_D": _w((lambda *s: _rng.normal(s) * 0.05)(D)),
        }
    _A_in = _A_setup()

    def _B_setup():
        B, S, D = 1, 2048, 1024
        return {
            "x": _w((lambda *s: _rng.normal(s) * 0.05)(B, S, D)),
            "wqkv": _w((lambda *s: _rng.normal(s) * 0.05)(D, 3 * D)),
            "wo": _w((lambda *s: _rng.normal(s) * 0.05)(D, D)),
        }
    _B_in = _B_setup()

    return {
        "A_q": _A_in["q"],
        "A_k": _A_in["k"],
        "A_v": _A_in["v"],
        "A_shift_k": _A_in["shift_k"],
        "A_ssm_k": _A_in["ssm_k"],
        "A_ssm_D": _A_in["ssm_D"],
        "B_x": _B_in["x"],
        "B_wqkv": _B_in["wqkv"],
        "B_wo": _B_in["wo"],
    }

def reference(A_q, A_k, A_v, A_shift_k, A_ssm_k, A_ssm_D, B_x, B_wqkv, B_wo):
    def _A_ref(q, k, v, shift_k, ssm_k, ssm_D):
        B, S, D = q.shape
        ks = shift_k.shape[-1]
        k_pad = jnp.pad(k, ((0, 0), (ks - 1, 0), (0, 0)))
        k_shift = jnp.zeros_like(k)
        for t in range(ks):
            k_shift = k_shift + k_pad[:, t:t + S, :] * shift_k[:, ks - 1 - t][None, None, :]
        kv = k_shift * v
        L = 2 * S
        kv_pad = jnp.pad(kv, ((0, 0), (0, S), (0, 0)))
        kf_pad = jnp.pad(ssm_k, ((0, 0), (0, S)))
        kv_f = (lambda x, axes=(-2,-1): jnp.fft.rfft2(x.astype(jnp.float32), axes=axes))(kv_pad[:, None, :, :], axes=(1, 2))
        kf_f = (lambda x, axes=(-2,-1): jnp.fft.rfft2(x.astype(jnp.float32), axes=axes))(kf_pad[:, None, :], axes=(1, 2))
        kf_f = (lambda x, *d: x.transpose(*d))(kf_f, 1, 2, 0)
        y_f = kv_f * kf_f[None, :, :, :]
        y = (lambda x, s, axes=(-2,-1): jnp.fft.irfft2(x, s=s, axes=axes).astype(jnp.bfloat16))(y_f, (1, L), axes=(1, 2))[:, 0, :S, :]
        y = y + kv * ssm_D[None, None, :]
        return q * y

    def _B_ref(x, wqkv, wo):
        B, S, D = x.shape
        H = 32; Dh = D // H
        qkv = (lambda x, *d: x.transpose(*d))((x @ wqkv).reshape(B, S, 3, H, Dh), 2, 0, 3, 1, 4)
        q, k, v = qkv[0], qkv[1], qkv[2]
        phi = lambda t: jnp.where(t > 0, t + 1, jnp.exp(t)) + 1e-6
        pq, pk = phi(q), phi(k)
        kv = jnp.einsum("bhsd,bhse->bhde", pk, v)
        z = jnp.einsum("bhsd->bhd", pk)
        num = jnp.einsum("bhqd,bhde->bhqe", pq, kv)
        den = jnp.einsum("bhqd,bhd->bhq", pq, z)[..., None] + 1e-6
        o = num / den
        return (lambda x, *d: x.transpose(*d))(o, 0, 2, 1, 3).reshape(B, S, D) @ wo

    a = _A_ref(A_q, A_k, A_v, A_shift_k, A_ssm_k, A_ssm_D)
    b = _B_ref(B_x, B_wqkv, B_wo)
    return jnp.concatenate([a, b], axis=-1)
```

```python
import jax
import jax.numpy as jnp
import numpy as np
import jax.experimental.pallas as pl
import jax.experimental.pallas.tpu as pltpu

S, D, DH = 2048, 1024, 32
CT = 128
RB = 512
NC = 128
RS = 8
BF, F32, U32 = jnp.bfloat16, jnp.float32, jnp.uint32


def _pack_rows(a):
    u = np.ascontiguousarray(a, np.float32).view(np.uint32).astype(np.uint64)
    u = ((u + 0x7FFF + ((u >> 16) & 1)) >> 16).astype(np.uint32)
    return u[..., 0::2, :] | (u[..., 1::2, :] << 16)


def _dft_constants():
    k1 = np.arange(128)
    n = 16 * k1[None, None, :] + np.arange(16)[:, None, None]
    th = 2 * np.pi * (k1[None, :, None] + 0.25) * n / S
    g = np.concatenate([np.cos(th), np.sin(th)], 1)
    gt = np.stack([np.cos(th), np.sin(th)], 2) / S
    gt = gt.reshape(16, 256, 128).transpose(0, 2, 1)
    return _pack_rows(g), _pack_rows(gt)


_G, _GT = _dft_constants()


def _cmulw(x, e, sg):
    e = (e * sg) % 16
    r, i = x
    if e == 0:
        return x
    if e == 4:
        return (-i, r)
    if e == 12:
        return (i, -r)
    c, s = np.cos(np.pi * e / 8), np.sin(np.pi * e / 8)
    if e % 2 == 0:
        h = np.float32(abs(c))
        if c * s > 0:
            u, v = (r - i) * h, (r + i) * h
        else:
            u, v = (r + i) * h, (i - r) * h
        return (u, v) if c > 0 else (-u, -v)
    c, s = np.float32(c), np.float32(s)
    return (r * c - i * s, r * s + i * c)


def _dft4(x, sg):
    (ar, ai), (br, bi), (cr, ci), (dr, di) = x
    pr, pi_, qr, qi = ar + cr, ai + ci, ar - cr, ai - ci
    tr, ti, ur, ui = br + dr, bi + di, br - dr, bi - di
    o1, o3 = (qr - ui, qi + ur), (qr + ui, qi - ur)
    if sg < 0:
        o1, o3 = o3, o1
    return [(pr + tr, pi_ + ti), o1, (pr - tr, pi_ - ti), o3]


def _dft16(x, sg):
    t = [_dft4([x[4 * m + j] for m in range(4)], sg) for j in range(4)]
    out = [None] * 16
    for a in range(4):
        o = _dft4([_cmulw(t[j][a], a * j, sg) for j in range(4)], sg)
        for b in range(4):
            out[a + 4 * b] = o[b]
    return out


def _dot(a, b):
    return jnp.dot(a, b, preferred_element_type=F32)


def _bf(x):
    return pltpu.bitcast(x, BF)


def _pk(a, b):
    return pltpu.pack_elementwise([a, b], packed_dtype=BF)


def _phi(t):
    return jnp.where(t > 0, t + 1.0, jnp.exp(jnp.minimum(t, 0.0))) + 1e-6


def _interleave(ga, gb, wa, wb):
    tot = [float(wa), float(wb)]
    done, gens = [0.0, 0.0], [ga, gb]
    while gens[0] is not None or gens[1] is not None:
        live = [n for n in (0, 1) if gens[n] is not None]
        n = min(live, key=lambda t: done[t] / tot[t])
        w = next(gens[n], None)
        if w is None:
            gens[n] = None
        else:
            done[n] += w


def _kernel(q_h, k_h, v_h, sh_ref, d_ref, kk_h, x_h, w_h, wo_h, g_h, gt_h, o_h,
            qb, kb, vb, kkb, xb, wb, wob, gb, gtb, oab, obb,
            kpad, kvb, kvf, ktb, ax, ak, cs, ys, kvacc, zacc, mm, zm, pbuf, sd_ref,
            sa, sx, sw, sc, soa, sob):
    def a_in(i):
        col = pl.ds(pl.multiple_of(i * CT, CT), CT)
        return [pltpu.make_async_copy(k_h.at[:, col], kb.at[i], sa.at[0, i]),
                pltpu.make_async_copy(v_h.at[:, col], vb.at[i], sa.at[1, i]),
                pltpu.make_async_copy(kk_h.at[col, :], kkb.at[i], sa.at[2, i]),
                pltpu.make_async_copy(q_h.at[:, col], qb.at[i], sa.at[3, i])]

    def a_out(i):
        col = pl.ds(pl.multiple_of(i * CT, CT), CT)
        return pltpu.make_async_copy(oab.at[i], o_h.at[:, col], soa.at[i])

    def x_in(i):
        r = pl.ds(pl.multiple_of(i * RB, RB), RB)
        return pltpu.make_async_copy(x_h.at[r, :], xb.at[i], sx.at[i])

    def b_out(i, j):
        r = pl.ds(pl.multiple_of(i * RB, RB), RB)
        return pltpu.make_async_copy(obb.at[i, :, pl.ds(j * NC, NC)],
                                     o_h.at[r, pl.ds(D + j * NC, NC)], sob.at[i, j])

    def w_in(j):
        return pltpu.make_async_copy(w_h.at[:, pl.ds(j * D, D)], wb.at[j], sw.at[j])

    wo_in = pltpu.make_async_copy(wo_h, wob, sw.at[1])
    c_in = [pltpu.make_async_copy(g_h, gb, sc.at[1]),
            pltpu.make_async_copy(gt_h, gtb, sc.at[2])]

    def wc_in(j, n):
        c = pl.ds(n * NC, NC)
        return pltpu.make_async_copy(
            w_h.at[:, pl.ds(j * D + n * NC, NC)], wb.at[j, :, c], sw.at[8 * j + n])

    def start(cs_):
        for c in cs_:
            c.start()

    def wait(cs_):
        for c in cs_:
            c.wait()

    def fwd1(src, dst):
        for j in range(4):
            o = [_dot(_bf(gb[4 * m + j]),
                      src[pl.ds(4 * m + j, 128, stride=17), :].astype(BF))
                 for m in range(4)]
            t = _dft4([(u[:128], u[128:]) for u in o], 1)
            for a in range(4):
                r, im = _cmulw(t[a], a * j, 1)
                dst[4 * a + j, pl.ds(0, 128), :] = r
                dst[4 * a + j, pl.ds(128, 128), :] = im
            yield 2

    def ld4(ref, gs, r):
        return [(ref[g, pl.ds(r, RS), :], ref[g, pl.ds(128 + r, RS), :]) for g in gs]

    def gen_a(i):
        kt = kkb[i].T.astype(F32)
        for n in range(128):
            ktb[pl.ds(17 * n, 16), :] = kt[16 * n:16 * n + 16]
        yield 4
        yield from fwd1(ktb, ak)
        sd = sd_ref[i, pl.ds(0, 5), :]
        kpad[pl.ds(0, 8), :] = jnp.zeros((8, CT), F32)
        kpad[pl.ds(8, S), :] = kb[i].astype(F32)
        for n in range(32):
            ks = None
            for t in range(4):
                term = kpad[pl.ds(64 * n + 5 + t, 64), :] * sd[3 - t:4 - t, :]
                ks = term if ks is None else ks + term
            kv = (ks * vb[i, pl.ds(64 * n, 64), :].astype(F32)).astype(BF)
            kvf[pl.ds(64 * n, 64), :] = kv.astype(F32) * sd[4:5, :]
            kv = kv.astype(F32)
            for m in range(4):
                kvb[pl.ds(17 * (4 * n + m), 16), :] = kv[16 * m:16 * m + 16]
            if n % 4 == 3:
                yield 12
        yield from fwd1(kvb, ax)
        for a in range(4):
            gs = [4 * a + j for j in range(4)]
            for r in range(0, 128, RS):
                y = [(xr * kr - xi * ki, xr * ki + xi * kr) for (xr, xi), (kr, ki)
                     in zip(_dft4(ld4(ax, gs, r), 1), _dft4(ld4(ak, gs, r), 1))]
                for j, t in enumerate(_dft4(y, -1)):
                    u, w = _cmulw(t, a * j, -1)
                    ax[4 * a + j, pl.ds(r, RS), :] = u
                    ax[4 * a + j, pl.ds(128 + r, RS), :] = w
                if r % 32 == 32 - RS:
                    yield 10
        for j in range(4):
            gs = [4 * a + j for a in range(4)]
            for r in range(0, 128, RS):
                for m, (u, w) in enumerate(_dft4(ld4(ax, gs, r), -1)):
                    cs[4 * m + j, pl.ds(r, RS), :] = _pk(u, w)
            yield 8
        for g in range(16):
            ys[pl.ds(g, 128, stride=17), :] = _dot(_bf(gtb[g]), _bf(cs[g]))
            if g % 4 == 3:
                yield 1
        for n in range(32):
            sl = pl.ds(64 * n, 64)
            oab[i, sl, :] = (qb[i, sl, :].astype(F32)
                             * (jnp.concatenate(
                                 [ys[pl.ds(17 * (4 * n + m), 16), :] for m in range(4)], 0)
                                + kvf[sl, :])).astype(BF)
            if n % 8 == 7:
                yield 8

    def gen_b1(i, hook=lambda n: None):
        for j in range(D // NC):
            c = pl.ds(j * NC, NC)
            hook(2 * j)
            x = xb[i]
            pk = _phi(_dot(x, wb[1, :, c]))
            zacc[:, c] += jnp.sum(pk.reshape(RB // 8, 8, NC), axis=0)
            pk = pk.astype(BF)
            yield 1
            hook(2 * j + 1)
            v = _dot(x, wb[2, :, c]).astype(BF)
            for h in range(NC // 128):
                s = slice(128 * h, 128 * h + 128)
                kvacc[j * (NC // 128) + h] += jax.lax.dot_general(
                    pk[:, s], v[:, s], (((0,), (0,)), ((), ())),
                    preferred_element_type=F32)
            yield 1

    def mid():
        r = jax.lax.broadcasted_iota(jnp.int32, (128, 128), 0) // DH
        c = jax.lax.broadcasted_iota(jnp.int32, (128, 128), 1) // DH
        same = r == c
        for j in range(D // 128):
            s = pl.ds(128 * j, 128)
            kv = jnp.where(same, kvacc[j], 0.0).astype(BF)
            mm[s, :] = _dot(kv, wob[s, :]).astype(BF)
            z = jnp.sum(zacc[:, s], axis=0, keepdims=True)
            zm[j] = jnp.where(same, jnp.broadcast_to(z, (128, 128)).T, 0.0).astype(BF)

    def gen_b2(i):
        x = xb[i]
        for j in range(D // NC):
            pq = _phi(_dot(x, wb[0, :, pl.ds(j * NC, NC)]))
            pqb = pq.astype(BF)
            for h in range(NC // 128):
                s = slice(128 * h, 128 * h + 128)
                den = _dot(pqb[:, s], zm[j * (NC // 128) + h]) + 1e-6
                pbuf[:, pl.ds(j * NC + 128 * h, 128)] = (pq[:, s] / den).astype(BF)
            yield 1
        for j in range(D // NC):
            c = pl.ds(j * NC, NC)
            obb[i, :, c] = _dot(pbuf[...], mm[:, c]).astype(BF)
            b_out(i, j).start()
            yield 1

    a0 = a_in(0)
    wc = [wc_in(1 + n % 2, n // 2) for n in range(16)]
    start([x_in(0), wc[0]])
    kvacc[...] = jnp.zeros_like(kvacc)
    zacc[...] = jnp.zeros_like(zacc)
    dv = d_ref[...].astype(F32).reshape(1, D)
    for t in range(8):
        sd_ref[t, pl.ds(0, 4), :] = sh_ref[pl.ds(CT * t, CT), :].astype(F32).T
        sd_ref[t, pl.ds(4, 1), :] = dv[:, CT * t:CT * t + CT]
    feed = {0: wc[1:4] + [a0[2], c_in[0]], 1: wc[4:6] + a0[:2], 3: wc[6:10],
            4: wc[10:] + [], 6: [c_in[1], a0[3]], 9: a_in(1) + [x_in(1)]}
    need = {0: [x_in(0)], 3: [a0[2], c_in[0]], 5: a0[:2], 9: c_in[1:], 12: a0[3:]}

    def hook(n):
        wait(need.get(n, []) + [wc[n]])
        start(feed.get(n, []))

    gb0, ga0 = gen_b1(0, hook), gen_a(0)
    for nb, na in ((4, 5), (2, 6), (2, 6), (2, 4), (2, 4), (1, 6), (3, 15)):
        for _ in range(nb):
            next(gb0)
        for _ in range(na):
            next(ga0, None)
    a_out(0).start()

    def step1(i, _):
        start(a_in(i + 1))

        @pl.when(i < 3)
        def _():
            x_in(i + 1).start()

        @pl.when(i == 1)
        def _():
            w_in(0).start()

        @pl.when(i == 2)
        def _():
            wo_in.start()

        wait(a_in(i) + [x_in(i)])
        _interleave(gen_b1(i), gen_a(i), 16.5, 344)
        a_out(i).start()

    jax.lax.fori_loop(1, 4, step1, None)
    wo_in.wait()
    w_in(0).wait()
    mid()

    def step2(i, _):
        @pl.when(i < 3)
        def _():
            start(a_in(i + 5))

        wait(a_in(i + 4))
        _interleave(gen_b2(i), gen_a(i + 4), 16.5, 344)
        a_out(i + 4).start()

    jax.lax.fori_loop(0, 4, step2, None)
    for i in range(8):
        a_out(i).wait()
    for i in range(4):
        for j in range(D // NC):
            b_out(i, j).wait()


@jax.jit
def pallas_concat_heads__ssm_conv_h3__linear_attn_block__prompt_kernel(
        A_q, A_k, A_v, A_shift_k, A_ssm_k, A_ssm_D, B_x, B_wqkv, B_wo):
    hbm = pl.BlockSpec(memory_space=pl.ANY)
    vm = pltpu.VMEM
    dma = pltpu.SemaphoreType.DMA
    tile = vm((8, S, CT), BF)
    out = pl.pallas_call(
        _kernel,
        in_specs=[hbm, hbm, hbm, *[pl.BlockSpec(memory_space=pltpu.VMEM)] * 2] + [hbm] * 6,
        out_specs=hbm,
        out_shape=jax.ShapeDtypeStruct((S, 2 * D), BF),
        scratch_shapes=[
            tile, tile, tile, vm((8, CT, S), BF), vm((4, RB, D), BF),
            vm((3, D, D), BF), vm((D, D), BF), vm(_G.shape, U32),
            vm(_GT.shape, U32), tile, vm((4, RB, D), BF),
            vm((S + 8, CT), F32), vm((17 * 128, CT), F32), vm((S, CT), F32),
            vm((17 * 128, CT), F32), vm((16, 256, CT), F32), vm((16, 256, CT), F32),
            vm((16, 128, CT), U32), vm((17 * 128, CT), F32),
            vm((8, 128, 128), F32), vm((8, D), F32), vm((D, D), BF),
            vm((8, 128, 128), BF), vm((RB, D), BF), vm((8, 8, CT), F32),
            dma((4, 8)), dma((4,)), dma((24,)), dma((3,)), dma((8,)), dma((4, 8))],
        compiler_params=pltpu.CompilerParams(vmem_limit_bytes=100 * 2**20),
    )(A_q[0], A_k[0], A_v[0], A_shift_k, A_ssm_D, A_ssm_k, B_x[0], B_wqkv, B_wo, _G, _GT)
    return out[None]
```
